```python
import os as _os
_os.environ.setdefault("JAX_PLATFORMS", "cpu")
import jax
import jax.numpy as jnp

def _softmax(x, axis=-1):
    return jax.nn.softmax(x, axis=axis)
def _gelu(x):
    return jax.nn.gelu(x, approximate=True)
def _silu(x):
    return jax.nn.silu(x)
def _sigmoid(x):
    return jax.nn.sigmoid(x)
def _layernorm(x, axis=-1, eps=1e-5):
    m = jnp.mean(x, axis=axis, keepdims=True)
    v = jnp.var(x, axis=axis, keepdims=True)
    return (x - m) / jnp.sqrt(v + eps)
def _scatter_add(tgt, idx, src, axis=0):
    return tgt.at[idx].add(src)
def _segment_sum(src, seg, n):
    return jax.ops.segment_sum(src, seg, n)
class _Rng:
    def __init__(self, key):
        self._k = key
    def _next(self):
        self._k, sub = jax.random.split(self._k)
        return sub
    def normal(self, shape):
        return jax.random.normal(self._next(), shape, dtype=jnp.bfloat16)
    def randint(self, lo, hi, shape):
        return jax.random.randint(self._next(), shape, lo, hi, dtype=jnp.int32)
    def uniform(self, shape, lo=0.0, hi=1.0):
        return jax.random.uniform(self._next(), shape, jnp.bfloat16, lo, hi)
    def permutation(self, n):
        return jax.random.permutation(self._next(), n)


kernel_name = 'sequential_preLN__softmax_full_mha__mixer_channel_mlp__prompt'

def setup_inputs():
    _rng = _Rng(jax.random.key(int.from_bytes(__import__("os").urandom(4), "little")))
    _w = (lambda a: (lambda t: t.astype(jnp.bfloat16) if jnp.issubdtype(t.dtype, jnp.floating) else t)(jnp.asarray(a)))
    def _A_setup():
        B, S, D = 1, 2048, 1024
        return {
            "x": _w((lambda *s: _rng.normal(s) * 0.05)(B, S, D)),
            "wqkv": _w((lambda *s: _rng.normal(s) * 0.05)(D, 3 * D)),
            "wo": _w((lambda *s: _rng.normal(s) * 0.05)(D, D)),
        }
    _A_in = _A_setup()

    def _B_setup():
        B, S, D, F = 1, 2048, 1024, 3584
        return {
            "x": _w((lambda *s: _rng.normal(s) * 0.05)(B, S, D)),
            "w1": _w((lambda *s: _rng.normal(s) * 0.8)(D, F) * (D ** -0.5)),
            "b1": _w((lambda *s: _rng.normal(s) * 0.8)(F)),
            "w2": _w((lambda *s: _rng.normal(s) * 0.8)(F, D) * (F ** -0.5)),
            "b2": _w((lambda *s: _rng.normal(s) * 0.05)(D)),
        }
    _B_in = _B_setup()

    return {
        "A_x": _A_in["x"],
        "A_wqkv": _A_in["wqkv"],
        "A_wo": _A_in["wo"],
        "B_x": _B_in["x"],
        "B_w1": _B_in["w1"],
        "B_b1": _B_in["b1"],
        "B_w2": _B_in["w2"],
        "B_b2": _B_in["b2"],
    }

def reference(A_x, A_wqkv, A_wo, B_x, B_w1, B_b1, B_w2, B_b2):
    def _A_ref(x, wqkv, wo):
        B, S, D = x.shape
        H = 32; Dh = D // H
        qkv = (lambda x, *d: x.transpose(*d))((x @ wqkv).reshape(B, S, 3, H, Dh), 2, 0, 3, 1, 4)
        q, k, v = qkv[0], qkv[1], qkv[2]
        scale = Dh ** -0.5
        scores = jnp.einsum("bhqd,bhkd->bhqk", q, k) * scale
        p = _softmax(scores, axis=-1)
        o = jnp.einsum("bhqk,bhkd->bhqd", p, v)
        return (lambda x, *d: x.transpose(*d))(o, 0, 2, 1, 3).reshape(B, S, D) @ wo

    def _B_ref(x, w1, b1, w2, b2):
        y = _layernorm(x, axis=-1)
        h = _gelu(jnp.einsum("bsd,df->bsf", y, w1) + b1)
        return jnp.einsum("bsf,fd->bsd", h, w2) + b2

    x = A_x
    h = x + _A_ref(_layernorm(x, axis=-1), A_wqkv, A_wo)
    h2 = h + _B_ref(_layernorm(h, axis=-1), B_w1, B_b1, B_w2, B_b2)
    return h2
```

```python
import functools
import math

import jax
import jax.numpy as jnp
import jax.experimental.pallas as pl
import jax.experimental.pallas.tpu as pltpu

f32 = jnp.float32
bf16 = jnp.bfloat16
i32 = jnp.int32

S = 2048
D = 1024
H = 32
DH = D // H
F = 3584
L = 128
TB = 512
NB = S // TB
C = 128
NC = S // C
NG = D // L
MB = 128
HM = MB // 2
DHALF = D // 2
FHALF = F // 2
EPS = 1e-5

DEFAULT = dict(skew=2, R=64, lag=1, dep2=2, only=None, qvb=4)


def _ln(x):
    mu = jnp.mean(x, axis=-1, keepdims=True)
    xc = x - mu
    var = jnp.mean(xc * xc, axis=-1, keepdims=True)
    return xc * jax.lax.rsqrt(var + EPS)


def _gelu(a):
    c0 = math.sqrt(2.0 / math.pi)
    u = a * (c0 + (c0 * 0.044715) * (a * a))
    return (0.5 * a) * (1.0 + jnp.tanh(u))


def _dot(a, b):
    return jnp.dot(a, b, preferred_element_type=f32)


def _pack(x):
    return pltpu.bitcast(x.astype(bf16), i32)


def _unpack(w):
    return pltpu.bitcast(w, bf16)


def _split(w):
    return tuple(pltpu.unpack_elementwise(w, index=i, packed_dtype=bf16, unpacked_dtype=f32)
                 for i in range(2))


def _join(even, odd):
    return pltpu.bitcast(pltpu.pack_elementwise([even, odd], packed_dtype=bf16), i32)


def _tie(x, z):
    return jnp.maximum(x, jnp.minimum(x, z))


def _rows(start, n):
    if isinstance(start, int):
        return pl.ds(start, n)
    return pl.ds(pl.multiple_of(start, n), n)


def _wrows(start, n):
    return _rows(start // 2, n // 2)


def _lhs_terms(a11, a12, a21, a22):
    return (a11 + a22, a21 + a22, a11, a22, a11 + a12, a21 - a11, a12 - a22)


def _rhs_terms(b11, b12, b21, b22):
    return (b11 + b22, b11, b12 - b22, b21 - b11, b22, b11 + b12, b21 + b22)


def _block_product(lhs, rhs, fill):
    def prod(i):
        m = _dot(lhs(i), rhs(i))
        fill()
        return m

    m = prod(0)
    c11, c22 = m, m
    m = prod(1)
    c21, c22 = m, c22 - m
    m = prod(2)
    c12, c22 = m, c22 + m
    m = prod(3)
    c11, c21 = c11 + m, c21 + m
    m = prod(4)
    c11, c12 = c11 - m, c12 + m
    c22 = c22 + prod(5)
    c11 = c11 + prod(6)
    return c11, c12, c21, c22


class _Filler:
    def __init__(self, slots, *task_lists):
        self.slots = slots
        self.lists = task_lists
        self.done = 0

    def __call__(self):
        for tasks in self.lists:
            lo = (len(tasks) * self.done) // self.slots
            hi = (len(tasks) * (self.done + 1)) // self.slots
            for task in tasks[lo:hi]:
                task()
        self.done += 1
        assert self.done <= self.slots


def _kernel(x_hbm, wqkv_hbm, wo_hbm, w1_hbm, b1_hbm, w2_hbm, b2_hbm, out_hbm,
            x_v, wqkv_v, wo_v, w1_v, w2_v, b1_v, b2_v, b1_f, b2_f, pa_v, pb_v,
            act_v, wa_v, wqv_v, w1op_v, w2op_v, k_v, qt_v, vt_v, ot_v, s_v,
            sem_x, sem_w, sem_o, *, cfg):
    skew, R, lag, dep2 = cfg["skew"], cfg["R"], cfg["lag"], cfg["dep2"]
    only = cfg["only"]
    pp = (pa_v, pb_v)

    def on(name):
        return only is None or name in only

    scope = [None]

    def mark(name):
        if not cfg.get("scopes"):
            return
        if scope[0] is not None:
            scope[0].__exit__(None, None, None)
            scope[0] = None
        if name and (cfg["scopes"] is True or name in cfg["scopes"]):
            scope[0] = jax.named_scope(name)
            scope[0].__enter__()

    def x_copy(i):
        lo, hi = ((0, MB), (MB, 5 * MB), (5 * MB, S))[i]
        rows = pl.ds(lo, hi - lo)
        return pltpu.make_async_copy(x_hbm.at[rows, :], x_v.at[rows, :], sem_x.at[i])

    def wqkv_copy(i):
        cols = pl.ds(i * D, D)
        return pltpu.make_async_copy(wqkv_hbm.at[:, cols], wqkv_v.at[i], sem_w.at[i])

    def wo_copy():
        return pltpu.make_async_copy(wo_hbm, wo_v, sem_w.at[3])

    def w1_copy():
        return pltpu.make_async_copy(w1_hbm, w1_v, sem_w.at[4])

    def w2_copy():
        return pltpu.make_async_copy(w2_hbm, w2_v, sem_w.at[5])

    def b1_copy():
        return pltpu.make_async_copy(b1_hbm, b1_v.at[pl.ds(0, F)], sem_w.at[6])

    def b2_copy():
        return pltpu.make_async_copy(b2_hbm, b2_v.at[pl.ds(0, D)], sem_w.at[7])

    def out_copy(mb):
        rows = _rows(mb * MB, MB)
        return pltpu.make_async_copy(x_v.at[rows, :], out_hbm.at[rows, :], sem_o.at[mb])

    def weight_task(src, dst, r0, t, khalf, nhalf):
        def task():
            lo = slice(t * L, (t + 1) * L)
            hi = slice(nhalf + t * L, nhalf + (t + 1) * L)
            top, bot = _rows(r0, 16), _rows(khalf + r0, 16)
            words = [_pack(src[r, c]) for r in (top, bot) for c in (lo, hi)]
            even, odd = zip(*[_split(w) for w in words])
            terms = [_join(e, o) for e, o in zip(_rhs_terms(*even), _rhs_terms(*odd))]
            terms[1], terms[4] = words[0], words[3]
            for q, term in enumerate(terms):
                dst[q, _wrows(r0, 16), lo] = term
        return task

    def weight_tasks(src, dst, part, nparts, khalf, nhalf):
        n = khalf // nparts
        return [weight_task(src, dst, part * n + u * 16, t, khalf, nhalf)
                for u in range(n // 16) for t in range(nhalf // L)]

    def norm_task(load, blk, u, dsts):
        def task():
            top = [_ln(v) for v in load(blk * MB + u * 16)]
            bot = [_ln(v) for v in load(blk * MB + HM + u * 16)]
            even, odd = [_lhs_terms(t[:, :DHALF], t[:, DHALF:], b[:, :DHALF], b[:, DHALF:])
                         for t, b in zip(top, bot)]
            for q, (e, o) in enumerate(zip(even, odd)):
                w = _join(e, o)
                for dst, base in dsts:
                    dst[q, _wrows(base + u * 16, 16), :] = w
        return task

    def norm_tasks(load, blk, dsts):
        return [norm_task(load, blk, u, dsts) for u in range(HM // 16)]

    def load_x(r0):
        return _split(_pack(x_v[_rows(r0, 16), :]))

    def load_h(r0):
        r0 = r0 if isinstance(r0, int) else pl.multiple_of(r0, 16)
        return tuple(jnp.concatenate([s_v[t, pl.ds(r0 + p, 8, stride=2), :] for t in range(NG)], axis=1)
                     for p in range(2))

    def k_body(i, _):
        @pl.when(i == 1)
        def _():
            x_copy(2).wait()
            wo_copy().start()
            w1_copy().start()

        @pl.when(i == 2)
        def _():
            wqkv_copy(0).wait()
            wqkv_copy(2).wait()

        src = wqkv_v.at[jnp.where(i < 2, 1, 2 * (i - 2))]
        dst = wqv_v.at[jnp.where(i < 3, 0, 1)]
        wtasks = weight_tasks(src, dst, 0, 1, DHALF, DHALF)
        for u in range(4):
            blk = i * 4 + u
            nxt = jnp.minimum(blk + 1, S // MB - 1)
            fill = _Filler(28, wtasks[u * 32:(u + 1) * 32],
                           norm_tasks(load_x, nxt, ((pp[(u + 1) % 2], 0), (act_v, nxt * HM))))
            cur = pp[u % 2]
            for c in range(DHALF // L):
                c11, c12, c21, c22 = _block_product(
                    lambda q: _unpack(cur[q]),
                    lambda q: _unpack(wa_v[q, :, c * L:(c + 1) * L]), fill)
                rows = _wrows(blk * MB, MB)
                k_v[c, rows, :] = _pack(jnp.concatenate([c11, c21], axis=0))
                k_v[DHALF // L + c, rows, :] = _pack(jnp.concatenate([c12, c22], axis=0))
        return 0

    mark("p0_start")
    if on("k"):
        x_copy(0).start()
        wqkv_copy(1).start()
        x_copy(1).start()
        x_copy(0).wait()
        for task in norm_tasks(load_x, 0, ((pa_v, 0), (act_v, 0))):
            task()
        wqkv_copy(1).wait()
        x_copy(2).start()
        wqkv_copy(0).start()
        wqkv_copy(2).start()

        def wk_body(part, _):
            for task in weight_tasks(wqkv_v.at[1], wa_v, part, 8, DHALF, DHALF):
                task()
            return 0

        jax.lax.fori_loop(0, 8, wk_body, 0)
        x_copy(1).wait()
        mark("p1a")
        jax.lax.fori_loop(0, NB, k_body, 0)
        mark("p1b")
        wo_copy().wait()
        w1_copy().wait()
        w2_copy().start()
        b1_copy().start()
        b2_copy().start()

    qscale = (DH ** -0.5) * math.log2(math.e)
    QVB = cfg["qvb"]

    def qv_body(i, _):
        nparts = S // MB // QVB
        fill = _Filler(QVB * 56, weight_tasks(wo_v, wa_v, i, nparts, DHALF, DHALF),
                       weight_tasks(w1_v, w1op_v, i, nparts, DHALF, FHALF))
        for u in range(QVB):
            blk = i * QVB + u
            for which, dst in ((0, qt_v), (1, vt_v)):
                for c in range(DHALF // L):
                    c11, c12, c21, c22 = _block_product(
                        lambda q: _unpack(act_v[q, _wrows(blk * HM, HM), :]),
                        lambda q: _unpack(wqv_v[which, q, :, c * L:(c + 1) * L]), fill)
                    for half, (top, bot) in enumerate(((c11, c21), (c12, c22))):
                        r = jnp.concatenate([top, bot], axis=0)
                        if which == 0:
                            r = r * qscale
                        dst[blk, _wrows(half * DHALF + c * L, L), :] = _pack(r.astype(bf16).T)
        return 0

    if on("qv"):
        jax.lax.fori_loop(0, S // MB // QVB, qv_body, 0)

    def hs(g, j):
        return _wrows(g * L + j * DH, DH)

    def qweights(qb, g, j):
        parts = []
        if j > 0:
            parts.append(jnp.zeros((DH // 2 * j, TB), i32))
        parts.append(jnp.concatenate(
            [qt_v[qb * (TB // MB) + t, hs(g, j), :] for t in range(TB // MB)], axis=1))
        if j < 3:
            parts.append(jnp.zeros((DH // 2 * (3 - j), TB), i32))
        return _unpack(jnp.concatenate(parts, axis=0))

    def qk_chunk(g, qm, c, slot, m):
        s = _dot(_unpack(k_v[g, c * C // 2:(c + 1) * C // 2, :]), qm)
        for t in range(TB // L):
            s_v[slot * (TB // L) + t, c * C:(c + 1) * C, :] = s[:, t * L:(t + 1) * L]
        mc = jnp.max(s.reshape(C // 8, 8, TB), axis=0)
        return (mc if m is None else jnp.maximum(m, mc)), s

    def fin(m):
        return jnp.broadcast_to(jnp.max(m, axis=0, keepdims=True), (8, TB))

    NIT = NB * NG

    def att_body(it, carry):
        mcur, mpart = carry
        qb = it // NG
        g = it % NG
        itn = jnp.minimum(it + 1, NIT - 1)
        qbn = itn // NG
        gn = itn % NG

        def head(jj):
            return (qb, g, jj) if jj < 4 else (qbn, gn, jj - 4)

        shist = []
        for j in range(4):
            slot = j % 2
            q1 = head(j + 1)
            q2 = head(j + 2)
            qm1 = qweights(*q1)
            qm2 = qweights(*q2) if skew else None
            l = None
            acc = None
            mnext = None
            lhist = []
            for c in range(NC):
                cc = c + skew
                if cc < NC:
                    mpart, s = qk_chunk(q1[1], qm1, cc, 1 - slot, mpart)
                    if cc == NC - 1:
                        mnext = fin(mpart)
                        mpart = None
                else:
                    mpart, s = qk_chunk(q2[1], qm2, cc - NC, slot, mpart)
                shist.append(s)
                ps = []
                for r in range(C // R):
                    s = jnp.concatenate(
                        [s_v[slot * (TB // L) + t, c * C + r * R:c * C + (r + 1) * R, :]
                         for t in range(TB // L)], axis=1)
                    muse = mcur
                    if dep2 and len(shist) >= dep2:
                        muse = _tie(muse, shist[-dep2][r * R:r * R + 8])
                    if lag and len(lhist) >= lag:
                        muse = _tie(muse, lhist[-lag])
                    p = jnp.exp2(s.reshape(R // 8, 8, TB) - muse[None])
                    ls = jnp.sum(p, axis=0)
                    l = ls if l is None else l + ls
                    lhist.append(l)
                    ps.append(p.reshape(R, TB))
                pb = jnp.concatenate(ps, axis=0) if len(ps) > 1 else ps[0]
                pv = _dot(_unpack(vt_v[c, hs(g, j), :]), pb.astype(bf16))
                acc = pv if acc is None else acc + pv
            l = jnp.sum(l, axis=0, keepdims=True)
            o = _pack(acc * (1.0 / l))
            for t in range(TB // MB):
                ot_v[qb * (TB // MB) + t, hs(g, j), :] = o[:, t * MB:(t + 1) * MB]
            mcur = mnext
            if mpart is None:
                mpart = jnp.full((8, TB), -jnp.inf, f32)
        return mcur, mpart

    mark("p2pro")
    if on("att"):
        qm = qweights(0, 0, 0)
        m = None
        for c in range(NC):
            m, _ = qk_chunk(0, qm, c, 0, m)
        mcur0 = fin(m)
        qm = qweights(0, 0, 1)
        m = jnp.full((8, TB), -jnp.inf, f32)
        for c in range(skew):
            m, _ = qk_chunk(0, qm, c, 1, m)
        mark("p2")
        jax.lax.fori_loop(0, NIT, att_body, (mcur0, m))
    mark("p3a")
    if on("k"):
        w2_copy().wait()
        b1_copy().wait()
        b2_copy().wait()

    def o_task(blk, t, dst):
        def task():
            lo = _pack(_unpack(ot_v[blk, _wrows(t * L, L), :]).T)
            hi = _pack(_unpack(ot_v[blk, _wrows(DHALF + t * L, L), :]).T)
            words = (lo[:HM // 2], hi[:HM // 2], lo[HM // 2:], hi[HM // 2:])
            even, odd = zip(*[_split(w) for w in words])
            terms = [_join(e, o) for e, o in zip(_lhs_terms(*even), _lhs_terms(*odd))]
            terms[2], terms[3] = words[0], words[3]
            for q, term in enumerate(terms):
                dst[q, :, t * L:(t + 1) * L] = term
        return task

    def o_tasks(blk, dst):
        return [o_task(blk, t, dst) for t in range(DHALF // L)]

    def wo_body(i, _):
        wtasks = weight_tasks(w2_v, w2op_v, i, NB, FHALF, DHALF)
        for u in range(4):
            blk = i * 4 + u
            nxt = jnp.minimum(blk + 1, S // MB - 1)
            prv = jnp.maximum(blk - 1, 0)
            fill = _Filler(28, o_tasks(nxt, pp[(u + 1) % 2]),
                           norm_tasks(load_h, prv, ((act_v, prv * HM),)),
                           wtasks[u * 28:(u + 1) * 28])
            cur = pp[u % 2]
            res = []
            for c in range(DHALF // L):
                res.append(_block_product(
                    lambda q: _unpack(cur[q]),
                    lambda q: _unpack(wa_v[q, :, c * L:(c + 1) * L]), fill))
            rows = _rows(blk * MB, MB)
            for c, (c11, c12, c21, c22) in enumerate(res):
                cols = slice(c * L, (c + 1) * L)
                hcols = slice(DHALF + c * L, DHALF + (c + 1) * L)
                s_v[c, rows, :] = x_v[rows, cols].astype(f32) + jnp.concatenate([c11, c21], axis=0)
                s_v[NG // 2 + c, rows, :] = x_v[rows, hcols].astype(f32) + jnp.concatenate([c12, c22], axis=0)
        return 0

    if on("wo"):
        for task in o_tasks(0, pa_v):
            task()
        jax.lax.fori_loop(0, NB, wo_body, 0)
        last = S // MB - 1
        for task in norm_tasks(load_h, last, ((act_v, last * HM),)):
            task()

    mark("p3b")

    def mlp_body(mb, _):
        gs = []
        for c in range(FHALF // L):
            c11, c12, c21, c22 = _block_product(
                lambda q: _unpack(act_v[q, _wrows(mb * HM, HM), :]),
                lambda q: _unpack(w1op_v[q, :, c * L:(c + 1) * L]), lambda: None)
            blo = b1_f[:, c * L:(c + 1) * L]
            bhi = b1_f[:, FHALF + c * L:FHALF + (c + 1) * L]
            terms = _lhs_terms(_gelu(c11 + blo), _gelu(c12 + bhi), _gelu(c21 + blo), _gelu(c22 + bhi))
            gs.append([_pack(t) for t in terms])
        o11, o12, o21, o22 = _block_product(
            lambda q: _unpack(jnp.concatenate([g[q] for g in gs], axis=1)),
            lambda q: _unpack(w2op_v[q]), lambda: None)
        rows = _rows(mb * MB, MB)
        for half, (top, bot) in enumerate(((o11, o21), (o12, o22))):
            cols = slice(half * DHALF, (half + 1) * DHALF)
            o = jnp.concatenate([top, bot], axis=0) + b2_f[:, cols]
            h = jnp.concatenate([s_v[half * (NG // 2) + t, rows, :] for t in range(NG // 2)], axis=1)
            x_v[rows, cols] = (h + o).astype(bf16)
        out_copy(mb).start()
        return 0

    if on("mlp"):
        b1_f[:, 0:F] = b1_v[pl.ds(0, F)].astype(f32).reshape(1, F)
        b2_f[...] = b2_v[pl.ds(0, D)].astype(f32).reshape(1, D)
        jax.lax.fori_loop(0, S // MB, mlp_body, 0)
        mark("p4")
        for mb in range(S // MB):
            out_copy(mb).wait()
    mark(None)


def build(cfg=None, name="fused"):
    c = dict(DEFAULT)
    c.update(cfg or {})

    def fn(A_x, A_wqkv, A_wo, B_x, B_w1, B_b1, B_w2, B_b2):
        del B_x
        x = A_x.reshape(S, D)
        any_spec = pl.BlockSpec(memory_space=pl.ANY)
        out = pl.pallas_call(
            functools.partial(_kernel, cfg=c),
            out_shape=jax.ShapeDtypeStruct((S, D), bf16),
            in_specs=[any_spec] * 7,
            out_specs=any_spec,
            scratch_shapes=[
                pltpu.VMEM((S, D), bf16),
                pltpu.VMEM((3, D, D), bf16),
                pltpu.VMEM((D, D), bf16),
                pltpu.VMEM((D, F), bf16),
                pltpu.VMEM((F, D), bf16),
                pltpu.VMEM((4096,), bf16),
                pltpu.VMEM((2048,), bf16),
                pltpu.VMEM((1, 4096), f32),
                pltpu.VMEM((1, D), f32),
                pltpu.VMEM((7, HM // 2, DHALF), i32),
                pltpu.VMEM((7, HM // 2, DHALF), i32),
                pltpu.VMEM((7, S // 4, DHALF), i32),
                pltpu.VMEM((7, DHALF // 2, DHALF), i32),
                pltpu.VMEM((2, 7, DHALF // 2, DHALF), i32),
                pltpu.VMEM((7, DHALF // 2, FHALF), i32),
                pltpu.VMEM((7, FHALF // 2, DHALF), i32),
                pltpu.VMEM((NG, S // 2, L), i32),
                pltpu.VMEM((S // MB, D // 2, MB), i32),
                pltpu.VMEM((S // MB, D // 2, MB), i32),
                pltpu.VMEM((S // MB, D // 2, MB), i32),
                pltpu.VMEM((NG, S, L), f32),
                pltpu.SemaphoreType.DMA((3,)),
                pltpu.SemaphoreType.DMA((8,)),
                pltpu.SemaphoreType.DMA((S // MB,)),
            ],
            compiler_params=pltpu.CompilerParams(vmem_limit_bytes=112 * 1024 * 1024),
            name=name,
        )(x, A_wqkv, A_wo, B_w1, B_b1, B_w2, B_b2)
        return out.reshape(1, S, D)

    return fn


@jax.jit
def pallas_sequential_preLN__softmax_full_mha__mixer_channel_mlp__prompt_kernel(
    A_x, A_wqkv, A_wo, B_x, B_w1, B_b1, B_w2, B_b2
):
    return build()(A_x, A_wqkv, A_wo, B_x, B_w1, B_b1, B_w2, B_b2)
```

```python
import functools
import math

import jax
import jax.numpy as jnp
import jax.experimental.pallas as pl
import jax.experimental.pallas.tpu as pltpu

f32 = jnp.float32
bf16 = jnp.bfloat16
i32 = jnp.int32

S = 2048
D = 1024
DH = 32
F = 3584
EPS = 1e-5
L = 128
NG = D // L

MB = 128
HM = MB // 2
NMB = S // MB
DHALF = D // 2
FHALF = F // 2
SPARE = NMB

TB = 512
C = 128
NC = S // C
HEADS_PER_STEP = 8
SKEW = 2
R = 64

QV_BLOCKS = 2
NPART = NMB // QV_BLOCKS

WQ = 0
WV = WQ + DHALF // 2
W1 = WV + DHALF // 2
W2 = W1 + 4 * (DHALF // 2)
ARENA = W2 + FHALF // 2


def _dot(a, b):
    return jnp.dot(a, b, preferred_element_type=f32)


def _gelu(a):
    c0 = math.sqrt(2.0 / math.pi)
    u = a * (c0 + (c0 * 0.044715) * (a * a))
    return (0.5 * a) * (1.0 + jnp.tanh(u))


def _pack(x):
    return pltpu.bitcast(x.astype(bf16), i32)


def _unpack(w):
    return pltpu.bitcast(w, bf16)


def _split(w):
    return tuple(pltpu.unpack_elementwise(w, index=i, packed_dtype=bf16, unpacked_dtype=f32)
                 for i in range(2))


def _join(even, odd):
    return pltpu.bitcast(pltpu.pack_elementwise([even, odd], packed_dtype=bf16), i32)


def _rows(start, n):
    if isinstance(start, int):
        return pl.ds(start, n)
    return pl.ds(pl.multiple_of(start, n), n)


def _wrows(start, n):
    return _rows(start // 2, n // 2)


def _tile(t):
    return slice(t * L, (t + 1) * L)


def _after(w, zero):
    if zero is None:
        return w
    return pltpu.bitcast(pltpu.bitcast(w, i32) | zero, w.dtype)


def _tie(x, z):
    return jnp.maximum(x, jnp.minimum(x, z))


def _lhs_terms(a11, a12, a21, a22):
    return (a11 + a22, a21 + a22, a11, a22, a11 + a12, a21 - a11, a12 - a22)


def _rhs_terms(b11, b12, b21, b22):
    return (b11 + b22, b11, b12 - b22, b21 - b11, b22, b11 + b12, b21 + b22)


def _block_product(lhs, rhs, fill=None, sink=None):
    def prod(q):
        m = _dot(lhs(q), rhs(q))
        if fill is not None:
            fill(m)
        return m

    def done(row_half, col_half, value):
        if sink is not None:
            sink(row_half, col_half, value)

    c22 = prod(5)
    m = prod(1)
    c21, c22 = m, c22 - m
    m = prod(2)
    c12, c22 = m, c22 + m
    m = prod(0)
    c11, c22 = m, c22 + m
    done(1, 1, c22)
    m = prod(3)
    c11, c21 = c11 + m, c21 + m
    done(1, 0, c21)
    m = prod(4)
    c11, c12 = c11 - m, c12 + m
    done(0, 1, c12)
    c11 = c11 + prod(6)
    done(0, 0, c11)
    return c11, c12, c21, c22


class _Filler:
    def __init__(self, history, *lists):
        self.history = history
        self.lists = lists
        self.slot = 0

    def _zero(self, lag):
        if lag < 0 or lag >= len(self.history):
            return None
        z = self.history[-1 - lag]
        return jnp.where(z != z, 1, 0)

    def __call__(self, product):
        self.history.append(product[0:8, 0:L])
        for first, last, tasks in self.lists:
            n = last - first
            lo = (len(tasks) * min(max(self.slot - first, 0), n)) // n
            hi = (len(tasks) * min(max(self.slot + 1 - first, 0), n)) // n
            for lag, task in tasks[lo:hi]:
                task(self._zero(lag))
        self.slot += 1


def _kernel(x_hbm, wqkv_hbm, wo_hbm, w1_hbm, b1_hbm, w2_hbm, b2_hbm, out_hbm,
            x_v, wqkv_v, wo_v, w1_v, w2_v, b1_v, b2_v, b1_f, b2_f,
            act_v, arena_v, pa_v, pb_v, wa_v, ha_v, hb_v, late_v,
            k_v, qt_v, vt_v, ot_v, s_v, h_v,
            sem_x, sem_w, sem_out, sem_w1, sem_wo):
    pp = (pa_v, pb_v)
    hh = (ha_v, hb_v)

    def x_copy(i):
        lo, hi = ((0, 1), (1, 5), (5, 9), (9, 13), (13, NMB))[i]
        rows = pl.ds(lo * MB, (hi - lo) * MB)
        return pltpu.make_async_copy(x_hbm.at[rows, :], x_v.at[rows, :], sem_x.at[i])

    def wqkv_copy(i):
        return pltpu.make_async_copy(wqkv_hbm.at[:, pl.ds(i * D, D)], wqkv_v.at[i], sem_w.at[i])

    def w2_copy():
        return pltpu.make_async_copy(w2_hbm, w2_v, sem_w.at[3])

    def b1_copy():
        return pltpu.make_async_copy(b1_hbm, b1_v.at[pl.ds(0, F)], sem_w.at[4])

    def b2_copy():
        return pltpu.make_async_copy(b2_hbm, b2_v.at[pl.ds(0, D)], sem_w.at[5])

    def part_copies(part):
        n = DHALF // NPART
        return [pltpu.make_async_copy(src.at[_rows(base + part * n, n), :],
                                      dst.at[_rows(base + part * n, n), :],
                                      sem.at[h * NPART + part])
                for src, dst, sem in ((w1_hbm, w1_v, sem_w1), (wo_hbm, wo_v, sem_wo))
                for h, base in enumerate((0, DHALF))]

    def out_copy(blk):
        rows = _rows(blk * MB, MB)
        return pltpu.make_async_copy(x_v.at[rows, :], out_hbm.at[rows, :], sem_out.at[blk])

    def weight_tasks(src, dst, base, part, nparts, khalf, nhalf, lag=-1):
        def task(r0, t, zero=None):
            top, bot = _rows(r0, 16), _rows(khalf + r0, 16)
            words = [_after(_pack(src[r, c]), zero)
                     for r in (top, bot) for c in (_tile(t), _tile(nhalf // L + t))]
            even, odd = zip(*[_split(w) for w in words])
            terms = [_join(e, o) for e, o in zip(_rhs_terms(*even), _rhs_terms(*odd))]
            terms[1], terms[4] = words[0], words[3]
            rows = _rows(base + (t // 4) * (khalf // 2) + r0 // 2, 8)
            for q, term in enumerate(terms):
                dst[q, rows, _tile(t % 4)] = term

        n = khalf // nparts
        return [(lag, functools.partial(task, part * n + u * 16, t))
                for u in range(n // 16) for t in range(nhalf // L)]

    def weight_terms(src, base, q, t):
        r0 = base + (t // 4) * (DHALF // 2)
        return _unpack(src[q, r0:r0 + DHALF // 2, _tile(t % 4)])

    def act_terms(q, blk):
        return _unpack(act_v[q, _rows(blk * (HM // 2), HM // 2), :])

    def norm_tasks(load, blk, dst, copy=None, lag=-1):
        tasks = []
        for u in range(HM // 16):
            stats = []

            def stat_task(zero=None, u=u, stats=stats):
                for r0 in (blk * MB + u * 16, blk * MB + HM + u * 16):
                    for v in zip(*[load(r0, t, zero) for t in range(NG)]):
                        v = jnp.concatenate(v, axis=1)
                        mu = jnp.mean(v, axis=-1, keepdims=True)
                        vc = v - mu
                        var = jnp.mean(vc * vc, axis=-1, keepdims=True)
                        stats.append((mu, jax.lax.rsqrt(var + EPS)))

            def tile_task(t, zero=None, u=u, stats=stats):
                quads = []
                for i, r0 in enumerate((blk * MB + u * 16, blk * MB + HM + u * 16)):
                    for tt in (t, NG // 2 + t):
                        quads.append([(v - mu) * rs for v, (mu, rs)
                                      in zip(load(r0, tt, zero), stats[2 * i:2 * i + 2])])
                even, odd = zip(*quads)
                rows = _rows(dst * (HM // 2) + u * 8, 8)
                for q, (e, o) in enumerate(zip(_lhs_terms(*even), _lhs_terms(*odd))):
                    w = _join(e, o)
                    act_v[q, rows, _tile(t)] = w
                    if copy is not None:
                        copy[q, u * 8:(u + 1) * 8, _tile(t)] = w

            tasks.append((-1, stat_task))
            tasks += [(lag, functools.partial(tile_task, t)) for t in range(NG // 2)]
        return tasks

    def load_x(r0, t, zero):
        return _split(_after(_pack(x_v[_rows(r0, 16), _tile(t)]), zero))

    def load_h(buf):
        def load(r0, t, zero):
            return tuple(_after(buf[t, pl.ds(r0 + p, 8, stride=2), :], zero) for p in range(2))
        return load

    def run(tasks):
        for _, task in tasks:
            task()

    x_copy(0).start()
    wqkv_copy(1).start()
    x_copy(1).start()
    hb_v[...] = jnp.zeros(hb_v.shape, f32)
    late_v[...] = jnp.zeros(late_v.shape, i32)
    x_copy(0).wait()
    run(norm_tasks(load_x, 0, 0, pa_v))
    wqkv_copy(1).wait()
    x_copy(2).start()
    wqkv_copy(0).start()

    def wk_body(part, _):
        run(weight_tasks(wqkv_v.at[1], wa_v, 0, part, 8, DHALF, DHALF))
        return 0

    jax.lax.fori_loop(0, 8, wk_body, 0)
    x_copy(1).wait()

    def k_body(i, _):
        @pl.when(i == 1)
        def _():
            x_copy(2).wait()
            x_copy(3).start()
            wqkv_copy(2).start()

        @pl.when(i == 2)
        def _():
            x_copy(3).wait()
            wqkv_copy(0).wait()
            x_copy(4).start()
            for cp in part_copies(0):
                cp.start()

        @pl.when(i == 3)
        def _():
            x_copy(4).wait()
            wqkv_copy(2).wait()
            for part in (1, 2):
                for cp in part_copies(part):
                    cp.start()

        wtasks = weight_tasks(wqkv_v.at[jnp.where(i < 2, 1, 2 * (i - 2))], arena_v,
                              jnp.where(i < 3, WQ, WV), 0, 1, DHALF, DHALF, lag=4)
        history = []
        for u in range(4):
            blk = i * 4 + u
            nxt = jnp.minimum(blk + 1, NMB - 1)
            fill = _Filler(history, (0, 26, wtasks[u * 32:(u + 1) * 32]),
                           (7, 26, norm_tasks(load_x, nxt, blk + 1, pp[(u + 1) % 2], lag=4)))
            for c in range(NG // 2):
                def sink(rh, ch, v):
                    k_v[ch * (NG // 2) + c, _wrows(blk * MB + rh * HM, HM), :] = _pack(v)

                _block_product(lambda q: _unpack(pp[u % 2][q]),
                               lambda q: weight_terms(wa_v, 0, q, c), fill, sink)
        return 0

    jax.lax.fori_loop(0, NMB // 4, k_body, 0)

    qscale = (DH ** -0.5) * math.log2(math.e)

    def flush_late(blk):
        for half in range(2):
            vt_v[blk, _wrows(half * DHALF + DHALF - L, L), :] = _pack(_unpack(late_v[half]).T)

    def qv_body(i, _):
        for cp in part_copies(i):
            cp.wait()

        @pl.when(i + 3 < NPART)
        def _():
            for cp in part_copies(i + 3):
                cp.start()

        slots = QV_BLOCKS * 56
        fill = _Filler([], (0, slots, weight_tasks(wo_v, wa_v, 0, i, NPART, DHALF, DHALF)),
                       (0, slots, weight_tasks(w1_v, arena_v, W1, i, NPART, DHALF, FHALF)))
        flush_late(jnp.where(i == 0, SPARE, i * QV_BLOCKS - 1))
        for u in range(QV_BLOCKS):
            blk = i * QV_BLOCKS + u
            for base, dst in ((WQ, qt_v), (WV, vt_v)):
                for c in range(NG // 2):
                    c11, c12, c21, c22 = _block_product(
                        lambda q: act_terms(q, blk),
                        lambda q: weight_terms(arena_v, base, q, c), fill)
                    for half, (top, bot) in enumerate(((c11, c21), (c12, c22))):
                        r = jnp.concatenate([top, bot], axis=0)
                        if base == WQ:
                            r = r * qscale
                        if u == QV_BLOCKS - 1 and base == WV and c == NG // 2 - 1:
                            late_v[half] = _pack(r)
                        else:
                            dst[blk, _wrows(half * DHALF + c * L, L), :] = _pack(r.astype(bf16).T)
        return 0

    jax.lax.fori_loop(0, NPART, qv_body, 0)
    flush_late(NMB - 1)

    w2_copy().start()
    b1_copy().start()
    b2_copy().start()

    def head_rows(g, j):
        return _wrows(g * L + j * DH, DH)

    def q_weights(qb, g, j):
        parts = []
        if j > 0:
            parts.append(jnp.zeros((DH // 2 * j, TB), i32))
        parts.append(jnp.concatenate(
            [qt_v[qb * (TB // MB) + t, head_rows(g, j), :] for t in range(TB // MB)], axis=1))
        if j < 3:
            parts.append(jnp.zeros((DH // 2 * (3 - j), TB), i32))
        return _unpack(jnp.concatenate(parts, axis=0))

    def scores(g, qw, c, slot, m):
        s = _dot(_unpack(k_v[g, c * C // 2:(c + 1) * C // 2, :]), qw)
        s_v[slot, c * C:(c + 1) * C, :] = s
        mc = jnp.max(s.reshape(C // 8, 8, TB), axis=0)
        return (mc if m is None else jnp.maximum(m, mc)), s

    def row_max(m):
        return jnp.broadcast_to(jnp.max(m, axis=0, keepdims=True), (8, TB))

    def att_body(it, carry):
        mcur, mpart = carry
        groups = HEADS_PER_STEP // 4

        def place(step):
            step = jnp.minimum(step, (S // TB) * NG - 1)
            return step // NG, step % NG

        places = [place(it * groups + e) for e in range(groups + 1)]

        def head(jj):
            return places[jj // 4] + (jj % 4,)

        recent = []
        for jj in range(HEADS_PER_STEP):
            qb, g, j = head(jj)
            slot = jj % 2
            h1, h2 = head(jj + 1), head(jj + 2)
            qw1, qw2 = q_weights(*h1), q_weights(*h2)
            l = acc = mnext = None
            for c in range(NC):
                ahead = c + SKEW
                if ahead < NC:
                    mpart, s = scores(h1[1], qw1, ahead, 1 - slot, mpart)
                    if ahead == NC - 1:
                        mnext, mpart = row_max(mpart), None
                else:
                    mpart, s = scores(h2[1], qw2, ahead - NC, slot, mpart)
                recent.append(s)
                ps = []
                for r in range(C // R):
                    s = s_v[slot, c * C + r * R:c * C + (r + 1) * R, :]
                    m = mcur
                    if len(recent) >= 3:
                        m = _tie(m, recent[-3][r * R + 56:r * R + 64])
                    if l is not None:
                        m = _tie(m, l)
                    p = jnp.exp2(s.reshape(R // 8, 8, TB) - m[None])
                    ls = jnp.sum(p, axis=0)
                    l = ls if l is None else l + ls
                    ps.append(p.reshape(R, TB))
                pt = jnp.concatenate(ps, axis=0)
                pv = _dot(_unpack(vt_v[c, head_rows(g, j), :]), pt.astype(bf16))
                acc = pv if acc is None else acc + pv
            l = jnp.sum(l, axis=0, keepdims=True)
            o = _pack(acc * (1.0 / l))
            for t in range(TB // MB):
                ot_v[qb * (TB // MB) + t, head_rows(g, j), :] = o[:, t * MB:(t + 1) * MB]
            mcur = mnext
        return mcur, mpart

    qw = q_weights(0, 0, 0)
    m = None
    for c in range(NC):
        m, _ = scores(0, qw, c, 0, m)
    m0 = row_max(m)
    qw = q_weights(0, 0, 1)
    m = jnp.full((8, TB), -jnp.inf, f32)
    for c in range(SKEW):
        m, _ = scores(0, qw, c, 1, m)
    jax.lax.fori_loop(0, (S // TB) * NG * 4 // HEADS_PER_STEP, att_body, (m0, m))

    w2_copy().wait()
    b1_copy().wait()
    b2_copy().wait()

    def o_tasks(blk, dst):
        def task(t, zero=None):
            lo = _pack(_unpack(ot_v[blk, _wrows(t * L, L), :]).T)
            hi = _pack(_unpack(ot_v[blk, _wrows(DHALF + t * L, L), :]).T)
            words = (lo[:HM // 2], hi[:HM // 2], lo[HM // 2:], hi[HM // 2:])
            even, odd = zip(*[_split(w) for w in words])
            terms = [_join(e, o) for e, o in zip(_lhs_terms(*even), _lhs_terms(*odd))]
            terms[2], terms[3] = words[0], words[3]
            for q, term in enumerate(terms):
                dst[q, :, _tile(t)] = term

        return [(-1, functools.partial(task, t)) for t in range(NG // 2)]

    def wo_body(i, _):
        wtasks = weight_tasks(w2_v, arena_v, W2, i, NMB // 4, FHALF, DHALF, lag=4)
        history = []
        for u in range(4):
            blk = i * 4 + u
            nxt = jnp.minimum(blk + 1, NMB - 1)
            fill = _Filler(history, (0, 28, o_tasks(nxt, pp[(u + 1) % 2])),
                           (7, 28, norm_tasks(load_h(hh[(u + 1) % 2]), 0,
                                              jnp.where(blk == 0, SPARE, blk - 1), lag=5)),
                           (0, 26, wtasks[u * 28:(u + 1) * 28]))
            for c in range(NG // 2):
                def sink(rh, ch, v):
                    rows = _rows(blk * MB + rh * HM, HM)
                    t = ch * (NG // 2) + c
                    h = x_v[rows, _tile(t)].astype(f32) + v
                    h_v[t, rows, :] = h
                    hh[u % 2][t, rh * HM:(rh + 1) * HM, :] = h

                _block_product(lambda q: _unpack(pp[u % 2][q]),
                               lambda q: weight_terms(wa_v, 0, q, c), fill, sink)
        return 0

    run(o_tasks(0, pa_v))
    jax.lax.fori_loop(0, NMB // 4, wo_body, 0)
    run(norm_tasks(load_h(hb_v), 0, NMB - 1))

    def mlp_body(blk, _):
        hidden = []
        for c in range(FHALF // L):
            c11, c12, c21, c22 = _block_product(
                lambda q: act_terms(q, blk), lambda q: weight_terms(arena_v, W1, q, c))
            blo, bhi = b1_f[:, _tile(c)], b1_f[:, _tile(FHALF // L + c)]
            terms = _lhs_terms(_gelu(c11 + blo), _gelu(c12 + bhi),
                               _gelu(c21 + blo), _gelu(c22 + bhi))
            hidden.append([_pack(t) for t in terms])
        o11, o12, o21, o22 = _block_product(
            lambda q: _unpack(jnp.concatenate([g[q] for g in hidden], axis=1)),
            lambda q: _unpack(arena_v[q, W2:W2 + FHALF // 2, :]))
        rows = _rows(blk * MB, MB)
        for half, (top, bot) in enumerate(((o11, o21), (o12, o22))):
            cols = slice(half * DHALF, (half + 1) * DHALF)
            o = jnp.concatenate([top, bot], axis=0) + b2_f[:, cols]
            h = jnp.concatenate([h_v[half * (NG // 2) + t, rows, :] for t in range(NG // 2)], axis=1)
            x_v[rows, cols] = (h + o).astype(bf16)
        out_copy(blk).start()
        return 0

    b1_f[:, 0:F] = b1_v[pl.ds(0, F)].astype(f32).reshape(1, F)
    b2_f[...] = b2_v[pl.ds(0, D)].astype(f32).reshape(1, D)
    jax.lax.fori_loop(0, NMB, mlp_body, 0)
    for blk in range(NMB):
        out_copy(blk).wait()


@jax.jit
def pallas_sequential_preLN__softmax_full_mha__mixer_channel_mlp__prompt_kernel(
    A_x: jax.Array,
    A_wqkv: jax.Array,
    A_wo: jax.Array,
    B_x: jax.Array,
    B_w1: jax.Array,
    B_b1: jax.Array,
    B_w2: jax.Array,
    B_b2: jax.Array,
):
    del B_x
    assert A_x.shape == (1, S, D) and B_w1.shape == (D, F)
    any_spec = pl.BlockSpec(memory_space=pl.ANY)
    out = pl.pallas_call(
        _kernel,
        out_shape=jax.ShapeDtypeStruct((S, D), bf16),
        in_specs=[any_spec] * 7,
        out_specs=any_spec,
        scratch_shapes=[
            pltpu.VMEM((S, D), bf16),
            pltpu.VMEM((3, D, D), bf16),
            pltpu.VMEM((D, D), bf16),
            pltpu.VMEM((D, F), bf16),
            pltpu.VMEM((F, D), bf16),
            pltpu.VMEM((4096,), bf16),
            pltpu.VMEM((2048,), bf16),
            pltpu.VMEM((1, 4096), f32),
            pltpu.VMEM((1, D), f32),
            pltpu.VMEM((7, (NMB + 1) * HM // 2, DHALF), i32),
            pltpu.VMEM((7, ARENA, DHALF), i32),
            pltpu.VMEM((7, HM // 2, DHALF), i32),
            pltpu.VMEM((7, HM // 2, DHALF), i32),
            pltpu.VMEM((7, DHALF // 2, DHALF), i32),
            pltpu.VMEM((NG, MB, L), f32),
            pltpu.VMEM((NG, MB, L), f32),
            pltpu.VMEM((2, MB // 2, L), i32),
            pltpu.VMEM((NG, S // 2, L), i32),
            pltpu.VMEM((NMB, D // 2, MB), i32),
            pltpu.VMEM((NMB + 1, D // 2, MB), i32),
            pltpu.VMEM((NMB, D // 2, MB), i32),
            pltpu.VMEM((2, S, TB), f32),
            pltpu.VMEM((NG, S, L), f32),
            pltpu.SemaphoreType.DMA((5,)),
            pltpu.SemaphoreType.DMA((6,)),
            pltpu.SemaphoreType.DMA((NMB,)),
            pltpu.SemaphoreType.DMA((2 * NPART,)),
            pltpu.SemaphoreType.DMA((2 * NPART,)),
        ],
        compiler_params=pltpu.CompilerParams(vmem_limit_bytes=118 * 1024 * 1024),
        name="preln_mha_mlp_block",
    )(A_x.reshape(S, D), A_wqkv, A_wo, B_w1, B_b1, B_w2, B_b2)
    return out.reshape(1, S, D)
```

```python
import functools
import math

import jax
import jax.numpy as jnp
import jax.experimental.pallas as pl
import jax.experimental.pallas.tpu as pltpu

f32 = jnp.float32
bf16 = jnp.bfloat16
i32 = jnp.int32

S = 2048
D = 1024
DH = 32
F = 3584
EPS = 1e-5
L = 128
NG = D // L

MB = 128
HM = MB // 2
NMB = S // MB
DHALF = D // 2
FHALF = F // 2
SPARE = NMB

TB = 512
C = 128
NC = S // C
HEADS_PER_STEP = 8
SKEW = 2
R = 64

QV_BLOCKS = 2
NPART = NMB // QV_BLOCKS

WQ = 0
WV = WQ + DHALF // 2
W1 = WV + DHALF // 2
W2 = W1 + 4 * (DHALF // 2)
ARENA = W2 + FHALF // 2


def _dot(a, b):
    return jnp.dot(a, b, preferred_element_type=f32)


def _gelu(a):
    c0 = math.sqrt(2.0 / math.pi)
    u = a * (c0 + (c0 * 0.044715) * (a * a))
    return (0.5 * a) * (1.0 + jnp.tanh(u))


def _pack(x):
    return pltpu.bitcast(x.astype(bf16), i32)


def _unpack(w):
    return pltpu.bitcast(w, bf16)


def _pack_all(xs):
    w = _pack(jnp.concatenate(xs, axis=1))
    n = xs[0].shape[1]
    return [w[:, i * n:(i + 1) * n] for i in range(len(xs))]


def _rows(start, n):
    if isinstance(start, int):
        return pl.ds(start, n)
    return pl.ds(pl.multiple_of(start, n), n)


def _wrows(start, n):
    return _rows(start // 2, n // 2)


def _tile(t):
    return slice(t * L, (t + 1) * L)


def _after(w, zero):
    if zero is None:
        return w
    return pltpu.bitcast(pltpu.bitcast(w, i32) | zero, w.dtype)


def _tie(x, z):
    return jnp.maximum(x, jnp.minimum(x, z))


def _lhs_terms(a11, a12, a21, a22):
    return (a11 + a22, a21 + a22, a11, a22, a11 + a12, a21 - a11, a12 - a22)


def _rhs_terms(b11, b12, b21, b22):
    return (b11 + b22, b11, b12 - b22, b21 - b11, b22, b11 + b12, b21 + b22)


def _block_product(lhs, rhs, fill=None, sink=None):
    def prod(q):
        m = _dot(lhs(q), rhs(q))
        if fill is not None:
            fill(m)
        return m

    def done(row_half, col_half, value):
        if sink is not None:
            sink(row_half, col_half, value)

    c22 = prod(5)
    m = prod(1)
    c21, c22 = m, c22 - m
    m = prod(2)
    c12, c22 = m, c22 + m
    m = prod(0)
    c11, c22 = m, c22 + m
    done(1, 1, c22)
    m = prod(3)
    c11, c21 = c11 + m, c21 + m
    done(1, 0, c21)
    m = prod(4)
    c11, c12 = c11 - m, c12 + m
    done(0, 1, c12)
    c11 = c11 + prod(6)
    done(0, 0, c11)
    return c11, c12, c21, c22


class _Filler:
    def __init__(self, history, *lists):
        self.history = history
        self.lists = lists
        self.slot = 0

    def _zero(self, lag):
        if lag < 0 or lag >= len(self.history):
            return None
        z = self.history[-1 - lag]
        return jnp.where(z != z, 1, 0)

    def __call__(self, product):
        self.history.append(product[0:8, 0:L])
        for first, last, tasks in self.lists:
            n = last - first
            lo = (len(tasks) * min(max(self.slot - first, 0), n)) // n
            hi = (len(tasks) * min(max(self.slot + 1 - first, 0), n)) // n
            for lag, task in tasks[lo:hi]:
                task(self._zero(lag))
        self.slot += 1


def _kernel(x_hbm, wqkv_hbm, wo_hbm, w1_hbm, b1_hbm, w2_hbm, b2_hbm, out_hbm,
            x_v, wqkv_v, wo_v, w1_v, w2_v, b1_v, b2_v, b1_f, b2_f,
            act_v, arena_v, pa_v, pb_v, wa_v, ha_v, hb_v, late_v,
            k_v, qt_v, vt_v, ot_v, s_v, h_v,
            sem_x, sem_w, sem_out, sem_w1, sem_wo):
    pp = (pa_v, pb_v)
    hh = (ha_v, hb_v)

    def x_copy(i):
        lo, hi = ((0, 1), (1, 5), (5, 9), (9, 13), (13, NMB))[i]
        rows = pl.ds(lo * MB, (hi - lo) * MB)
        return pltpu.make_async_copy(x_hbm.at[rows, :], x_v.at[rows, :], sem_x.at[i])

    def wqkv_copy(i):
        return pltpu.make_async_copy(wqkv_hbm.at[:, pl.ds(i * D, D)], wqkv_v.at[i], sem_w.at[i])

    def w2_copy():
        return pltpu.make_async_copy(w2_hbm, w2_v, sem_w.at[3])

    def b1_copy():
        return pltpu.make_async_copy(b1_hbm, b1_v.at[pl.ds(0, F)], sem_w.at[4])

    def b2_copy():
        return pltpu.make_async_copy(b2_hbm, b2_v.at[pl.ds(0, D)], sem_w.at[5])

    def part_copies(part):
        n = DHALF // NPART
        return [pltpu.make_async_copy(src.at[_rows(base + part * n, n), :],
                                      dst.at[_rows(base + part * n, n), :],
                                      sem.at[h * NPART + part])
                for src, dst, sem in ((w1_hbm, w1_v, sem_w1), (wo_hbm, wo_v, sem_wo))
                for h, base in enumerate((0, DHALF))]

    def out_copy(blk):
        rows = _rows(blk * MB, MB)
        return pltpu.make_async_copy(x_v.at[rows, :], out_hbm.at[rows, :], sem_out.at[blk])

    def weight_tasks(src, dst, base, part, nparts, khalf, nhalf, lag=-1):
        def task(r0, t, zero=None):
            top, bot = _rows(r0, 16), _rows(khalf + r0, 16)
            words = [_after(_pack(src[r, c]), zero)
                     for r in (top, bot) for c in (_tile(t), _tile(nhalf // L + t))]
            sums = _rhs_terms(*[_unpack(w).astype(f32) for w in words])
            t0, t2, t3, t5, t6 = _pack_all([sums[q] for q in (0, 2, 3, 5, 6)])
            terms = (t0, words[0], t2, t3, words[3], t5, t6)
            rows = _rows(base + (t // 4) * (khalf // 2) + r0 // 2, 8)
            for q, term in enumerate(terms):
                dst[q, rows, _tile(t % 4)] = term

        n = khalf // nparts
        return [(lag, functools.partial(task, part * n + u * 16, t))
                for u in range(n // 16) for t in range(nhalf // L)]

    def weight_terms(src, base, q, t):
        r0 = base + (t // 4) * (DHALF // 2)
        return _unpack(src[q, r0:r0 + DHALF // 2, _tile(t % 4)])

    def act_terms(q, blk):
        return _unpack(act_v[q, _rows(blk * (HM // 2), HM // 2), :])

    def norm_tasks(load, blk, dst, copy=None, lag=-1):
        tasks = []
        for u in range(HM // 16):
            stats = []

            def stat_task(zero=None, u=u, stats=stats):
                for r0 in (blk * MB + u * 16, blk * MB + HM + u * 16):
                    v = jnp.concatenate([load(r0, t, zero) for t in range(NG)], axis=1)
                    mu = jnp.mean(v, axis=-1, keepdims=True)
                    vc = v - mu
                    var = jnp.mean(vc * vc, axis=-1, keepdims=True)
                    stats.append((mu, jax.lax.rsqrt(var + EPS)))

            def tile_task(t, zero=None, u=u, stats=stats):
                quads = []
                for (mu, rs), r0 in zip(stats, (blk * MB + u * 16, blk * MB + HM + u * 16)):
                    for tt in (t, NG // 2 + t):
                        quads.append((load(r0, tt, zero) - mu) * rs)
                words = _pack_all(list(_lhs_terms(*quads)))
                rows = _rows(dst * (HM // 2) + u * 8, 8)
                for q, w in enumerate(words):
                    act_v[q, rows, _tile(t)] = w
                    if copy is not None:
                        copy[q, u * 8:(u + 1) * 8, _tile(t)] = w

            tasks.append((-1, stat_task))
            tasks += [(lag, functools.partial(tile_task, t)) for t in range(NG // 2)]
        return tasks

    def load_x(r0, t, zero):
        return _unpack(_after(_pack(x_v[_rows(r0, 16), _tile(t)]), zero)).astype(f32)

    def load_h(buf):
        def load(r0, t, zero):
            return jnp.concatenate(
                [_after(buf[t, pl.ds(r0 + 8 * p, 8), :], zero) for p in range(2)], axis=0)
        return load

    def run(tasks):
        for _, task in tasks:
            task()

    x_copy(0).start()
    wqkv_copy(1).start()
    x_copy(1).start()
    hb_v[...] = jnp.zeros(hb_v.shape, f32)
    late_v[...] = jnp.zeros(late_v.shape, i32)
    x_copy(0).wait()
    run(norm_tasks(load_x, 0, 0, pa_v))
    wqkv_copy(1).wait()
    x_copy(2).start()
    wqkv_copy(0).start()

    def wk_body(part, _):
        run(weight_tasks(wqkv_v.at[1], wa_v, 0, part, 8, DHALF, DHALF))
        return 0

    jax.lax.fori_loop(0, 8, wk_body, 0)
    x_copy(1).wait()

    def k_body(i, _):
        @pl.when(i == 1)
        def _():
            x_copy(2).wait()
            x_copy(3).start()
            wqkv_copy(2).start()

        @pl.when(i == 2)
        def _():
            x_copy(3).wait()
            wqkv_copy(0).wait()
            x_copy(4).start()
            for cp in part_copies(0):
                cp.start()

        @pl.when(i == 3)
        def _():
            x_copy(4).wait()
            wqkv_copy(2).wait()
            for part in (1, 2):
                for cp in part_copies(part):
                    cp.start()

        wtasks = weight_tasks(wqkv_v.at[jnp.where(i < 2, 1, 2 * (i - 2))], arena_v,
                              jnp.where(i < 3, WQ, WV), 0, 1, DHALF, DHALF, lag=4)
        history = []
        for u in range(4):
            blk = i * 4 + u
            nxt = jnp.minimum(blk + 1, NMB - 1)
            fill = _Filler(history, (0, 26, wtasks[u * 32:(u + 1) * 32]),
                           (2, 24, norm_tasks(load_x, nxt, blk + 1, pp[(u + 1) % 2], lag=6)))
            for c in range(NG // 2):
                def sink(rh, ch, v):
                    k_v[ch * (NG // 2) + c, _wrows(blk * MB + rh * HM, HM), :] = _pack(v)

                _block_product(lambda q: _unpack(pp[u % 2][q]),
                               lambda q: weight_terms(wa_v, 0, q, c), fill, sink)
        return 0

    jax.lax.fori_loop(0, NMB // 4, k_body, 0)

    qscale = (DH ** -0.5) * math.log2(math.e)

    def flush_late(blk):
        for half in range(2):
            vt_v[blk, _wrows(half * DHALF + DHALF - L, L), :] = _pack(_unpack(late_v[half]).T)

    def qv_body(i, _):
        for cp in part_copies(i):
            cp.wait()

        @pl.when(i + 3 < NPART)
        def _():
            for cp in part_copies(i + 3):
                cp.start()

        last = QV_BLOCKS * 56 - 14
        fill = _Filler(
            [], (0, last, weight_tasks(wo_v, wa_v, 0, i, NPART, DHALF, DHALF, lag=3)),
            (0, last, weight_tasks(w1_v, arena_v, W1, i, NPART, DHALF, FHALF, lag=3)))
        flush_late(jnp.where(i == 0, SPARE, i * QV_BLOCKS - 1))
        for u in range(QV_BLOCKS):
            blk = i * QV_BLOCKS + u
            for base, dst in ((WQ, qt_v), (WV, vt_v)):
                for c in range(NG // 2):
                    c11, c12, c21, c22 = _block_product(
                        lambda q: act_terms(q, blk),
                        lambda q: weight_terms(arena_v, base, q, c), fill)
                    for half, (top, bot) in enumerate(((c11, c21), (c12, c22))):
                        r = jnp.concatenate([top, bot], axis=0)
                        if base == WQ:
                            r = r * qscale
                        if u == QV_BLOCKS - 1 and base == WV and c == NG // 2 - 1:
                            late_v[half] = _pack(r)
                        else:
                            dst[blk, _wrows(half * DHALF + c * L, L), :] = _pack(r.astype(bf16).T)
        return 0

    jax.lax.fori_loop(0, NPART, qv_body, 0)
    flush_late(NMB - 1)

    w2_copy().start()
    b1_copy().start()
    b2_copy().start()

    def head_rows(g, j):
        return _wrows(g * L + j * DH, DH)

    def q_weights(qb, g, j):
        parts = []
        if j > 0:
            parts.append(jnp.zeros((DH // 2 * j, TB), i32))
        parts.append(jnp.concatenate(
            [qt_v[qb * (TB // MB) + t, head_rows(g, j), :] for t in range(TB // MB)], axis=1))
        if j < 3:
            parts.append(jnp.zeros((DH // 2 * (3 - j), TB), i32))
        return _unpack(jnp.concatenate(parts, axis=0))

    def scores(g, qw, c, slot, m):
        s = _dot(_unpack(k_v[g, c * C // 2:(c + 1) * C // 2, :]), qw)
        s_v[slot, c * C:(c + 1) * C, :] = s
        mc = jnp.max(s.reshape(C // 8, 8, TB), axis=0)
        return (mc if m is None else jnp.maximum(m, mc)), s

    def row_max(m):
        return jnp.broadcast_to(jnp.max(m, axis=0, keepdims=True), (8, TB))

    def att_body(it, carry):
        mcur, mpart = carry
        groups = HEADS_PER_STEP // 4

        def place(step):
            step = jnp.minimum(step, (S // TB) * NG - 1)
            return step // NG, step % NG

        places = [place(it * groups + e) for e in range(groups + 1)]

        def head(jj):
            return places[jj // 4] + (jj % 4,)

        recent = []
        for jj in range(HEADS_PER_STEP):
            qb, g, j = head(jj)
            slot = jj % 2
            h1, h2 = head(jj + 1), head(jj + 2)
            qw1, qw2 = q_weights(*h1), q_weights(*h2)
            l = acc = mnext = None
            for c in range(NC):
                ahead = c + SKEW
                if ahead < NC:
                    mpart, s = scores(h1[1], qw1, ahead, 1 - slot, mpart)
                    if ahead == NC - 1:
                        mnext, mpart = row_max(mpart), None
                else:
                    mpart, s = scores(h2[1], qw2, ahead - NC, slot, mpart)
                recent.append(s)
                ps = []
                for r in range(C // R):
                    s = s_v[slot, c * C + r * R:c * C + (r + 1) * R, :]
                    m = mcur
                    if len(recent) >= 3:
                        m = _tie(m, recent[-3][r * R + 56:r * R + 64])
                    if l is not None:
                        m = _tie(m, l)
                    p = jnp.exp2(s.reshape(R // 8, 8, TB) - m[None])
                    ls = jnp.sum(p, axis=0)
                    l = ls if l is None else l + ls
                    ps.append(p.reshape(R, TB))
                pt = jnp.concatenate(ps, axis=0)
                pv = _dot(_unpack(vt_v[c, head_rows(g, j), :]), pt.astype(bf16))
                acc = pv if acc is None else acc + pv
            l = jnp.sum(l, axis=0, keepdims=True)
            o = _pack(acc * (1.0 / l))
            for t in range(TB // MB):
                ot_v[qb * (TB // MB) + t, head_rows(g, j), :] = o[:, t * MB:(t + 1) * MB]
            mcur = mnext
        return mcur, mpart

    qw = q_weights(0, 0, 0)
    m = None
    for c in range(NC):
        m, _ = scores(0, qw, c, 0, m)
    m0 = row_max(m)
    qw = q_weights(0, 0, 1)
    m = jnp.full((8, TB), -jnp.inf, f32)
    for c in range(SKEW):
        m, _ = scores(0, qw, c, 1, m)
    jax.lax.fori_loop(0, (S // TB) * NG * 4 // HEADS_PER_STEP, att_body, (m0, m))

    w2_copy().wait()
    b1_copy().wait()
    b2_copy().wait()

    def o_tasks(blk, dst):
        def task(t, zero=None):
            lo = _pack(_unpack(ot_v[blk, _wrows(t * L, L), :]).T)
            hi = _pack(_unpack(ot_v[blk, _wrows(DHALF + t * L, L), :]).T)
            words = (lo[:HM // 2], hi[:HM // 2], lo[HM // 2:], hi[HM // 2:])
            sums = _lhs_terms(*[_unpack(w).astype(f32) for w in words])
            t0, t1, t4, t5, t6 = _pack_all([sums[q] for q in (0, 1, 4, 5, 6)])
            terms = (t0, t1, words[0], words[3], t4, t5, t6)
            for q, term in enumerate(terms):
                dst[q, :, _tile(t)] = term

        return [(-1, functools.partial(task, t)) for t in range(NG // 2)]

    def wo_body(i, _):
        wtasks = weight_tasks(w2_v, arena_v, W2, i, NMB // 4, FHALF, DHALF, lag=4)
        history = []
        for u in range(4):
            blk = i * 4 + u
            nxt = jnp.minimum(blk + 1, NMB - 1)
            fill = _Filler(history, (0, 28, o_tasks(nxt, pp[(u + 1) % 2])),
                           (7, 28, norm_tasks(load_h(hh[(u + 1) % 2]), 0,
                                              jnp.where(blk == 0, SPARE, blk - 1), lag=3)),
                           (0, 26, wtasks[u * 28:(u + 1) * 28]))
            for c in range(NG // 2):
                def sink(rh, ch, v):
                    rows = _rows(blk * MB + rh * HM, HM)
                    t = ch * (NG // 2) + c
                    h = x_v[rows, _tile(t)].astype(f32) + v
                    h_v[t, rows, :] = h
                    hh[u % 2][t, rh * HM:(rh + 1) * HM, :] = h

                _block_product(lambda q: _unpack(pp[u % 2][q]),
                               lambda q: weight_terms(wa_v, 0, q, c), fill, sink)
        return 0

    run(o_tasks(0, pa_v))
    jax.lax.fori_loop(0, NMB // 4, wo_body, 0)
    run(norm_tasks(load_h(hb_v), 0, NMB - 1))

    def mlp_body(blk, _):
        hidden = []
        for c in range(FHALF // L):
            c11, c12, c21, c22 = _block_product(
                lambda q: act_terms(q, blk), lambda q: weight_terms(arena_v, W1, q, c))
            blo, bhi = b1_f[:, _tile(c)], b1_f[:, _tile(FHALF // L + c)]
            terms = _lhs_terms(_gelu(c11 + blo), _gelu(c12 + bhi),
                               _gelu(c21 + blo), _gelu(c22 + bhi))
            hidden.append([_pack(t) for t in terms])
        o11, o12, o21, o22 = _block_product(
            lambda q: _unpack(jnp.concatenate([g[q] for g in hidden], axis=1)),
            lambda q: _unpack(arena_v[q, W2:W2 + FHALF // 2, :]))
        rows = _rows(blk * MB, MB)
        for half, (top, bot) in enumerate(((o11, o21), (o12, o22))):
            cols = slice(half * DHALF, (half + 1) * DHALF)
            o = jnp.concatenate([top, bot], axis=0) + b2_f[:, cols]
            h = jnp.concatenate([h_v[half * (NG // 2) + t, rows, :] for t in range(NG // 2)], axis=1)
            x_v[rows, cols] = (h + o).astype(bf16)
        out_copy(blk).start()
        return 0

    b1_f[:, 0:F] = b1_v[pl.ds(0, F)].astype(f32).reshape(1, F)
    b2_f[...] = b2_v[pl.ds(0, D)].astype(f32).reshape(1, D)
    jax.lax.fori_loop(0, NMB, mlp_body, 0)
    for blk in range(NMB):
        out_copy(blk).wait()


@jax.jit
def pallas_sequential_preLN__softmax_full_mha__mixer_channel_mlp__prompt_kernel(
    A_x: jax.Array,
    A_wqkv: jax.Array,
    A_wo: jax.Array,
    B_x: jax.Array,
    B_w1: jax.Array,
    B_b1: jax.Array,
    B_w2: jax.Array,
    B_b2: jax.Array,
):
    del B_x
    assert A_x.shape == (1, S, D) and B_w1.shape == (D, F)
    any_spec = pl.BlockSpec(memory_space=pl.ANY)
    out = pl.pallas_call(
        _kernel,
        out_shape=jax.ShapeDtypeStruct((S, D), bf16),
        in_specs=[any_spec] * 7,
        out_specs=any_spec,
        scratch_shapes=[
            pltpu.VMEM((S, D), bf16),
            pltpu.VMEM((3, D, D), bf16),
            pltpu.VMEM((D, D), bf16),
            pltpu.VMEM((D, F), bf16),
            pltpu.VMEM((F, D), bf16),
            pltpu.VMEM((4096,), bf16),
            pltpu.VMEM((2048,), bf16),
            pltpu.VMEM((1, 4096), f32),
            pltpu.VMEM((1, D), f32),
            pltpu.VMEM((7, (NMB + 1) * HM // 2, DHALF), i32),
            pltpu.VMEM((7, ARENA, DHALF), i32),
            pltpu.VMEM((7, HM // 2, DHALF), i32),
            pltpu.VMEM((7, HM // 2, DHALF), i32),
            pltpu.VMEM((7, DHALF // 2, DHALF), i32),
            pltpu.VMEM((NG, MB, L), f32),
            pltpu.VMEM((NG, MB, L), f32),
            pltpu.VMEM((2, MB // 2, L), i32),
            pltpu.VMEM((NG, S // 2, L), i32),
            pltpu.VMEM((NMB, D // 2, MB), i32),
            pltpu.VMEM((NMB + 1, D // 2, MB), i32),
            pltpu.VMEM((NMB, D // 2, MB), i32),
            pltpu.VMEM((2, S, TB), f32),
            pltpu.VMEM((NG, S, L), f32),
            pltpu.SemaphoreType.DMA((5,)),
            pltpu.SemaphoreType.DMA((6,)),
            pltpu.SemaphoreType.DMA((NMB,)),
            pltpu.SemaphoreType.DMA((2 * NPART,)),
            pltpu.SemaphoreType.DMA((2 * NPART,)),
        ],
        compiler_params=pltpu.CompilerParams(vmem_limit_bytes=118 * 1024 * 1024),
        name="preln_mha_mlp_block",
    )(A_x.reshape(S, D), A_wqkv, A_wo, B_w1, B_b1, B_w2, B_b2)
    return out.reshape(1, S, D)
```
